```python
import os as _os
_os.environ.setdefault("JAX_PLATFORMS", "cpu")
import jax
import jax.numpy as jnp

def _softmax(x, axis=-1):
    return jax.nn.softmax(x, axis=axis)
def _gelu(x):
    return jax.nn.gelu(x, approximate=True)
def _silu(x):
    return jax.nn.silu(x)
def _sigmoid(x):
    return jax.nn.sigmoid(x)
def _layernorm(x, axis=-1, eps=1e-5):
    m = jnp.mean(x, axis=axis, keepdims=True)
    v = jnp.var(x, axis=axis, keepdims=True)
    return (x - m) / jnp.sqrt(v + eps)
def _scatter_add(tgt, idx, src, axis=0):
    return tgt.at[idx].add(src)
def _segment_sum(src, seg, n):
    return jax.ops.segment_sum(src, seg, n)
class _Rng:
    def __init__(self, key):
        self._k = key
    def _next(self):
        self._k, sub = jax.random.split(self._k)
        return sub
    def normal(self, shape):
        return jax.random.normal(self._next(), shape, dtype=jnp.bfloat16)
    def randint(self, lo, hi, shape):
        return jax.random.randint(self._next(), shape, lo, hi, dtype=jnp.int32)
    def uniform(self, shape, lo=0.0, hi=1.0):
        return jax.random.uniform(self._next(), shape, jnp.bfloat16, lo, hi)
    def permutation(self, n):
        return jax.random.permutation(self._next(), n)


kernel_name = 'concat_heads__mha_block__ssm_conv_s4__prompt'

def setup_inputs():
    _rng = _Rng(jax.random.key(int.from_bytes(__import__("os").urandom(4), "little")))
    _w = (lambda a: (lambda t: t.astype(jnp.bfloat16) if jnp.issubdtype(t.dtype, jnp.floating) else t)(jnp.asarray(a)))
    def _A_setup():
        B, S, D, H = 1, 2048, 448, 16
        return {
            "x": _w((lambda *s: _rng.normal(s) * 0.2)(B, S, D)),
            "wqkv": _w((lambda *s: _rng.normal(s) * 0.2)(D, 3 * D)),
            "wo": _w((lambda *s: _rng.normal(s) * 0.05)(D, D)),
        }
    _A_in = _A_setup()

    def _B_setup():
        B, L, D, N = 1, 2048, 448, 256
        A_re = -jnp.exp((lambda *s: _rng.normal(s) * 0.2)(D, N))
        A_im = jnp.pi * (lambda *s: _rng.normal(s) * 0.2)(D, N)
        B_re = (lambda *s: _rng.normal(s) * 0.2)(D, N)
        B_im = (lambda *s: _rng.normal(s) * 0.2)(D, N)
        C_re = (lambda *s: _rng.normal(s) * 0.2)(D, N)
        C_im = (lambda *s: _rng.normal(s) * 0.2)(D, N)
        log_dt = (lambda *s: _rng.normal(s) * 0.2)(D) * 0.5 - 4.0
        Dskip = (lambda *s: _rng.normal(s) * 0.05)(D)
        return {
            "u": _w((lambda *s: _rng.normal(s) * 0.05)(B, L, D)),
            "A_re": _w(A_re),
            "A_im": _w(A_im),
            "B_re": _w(B_re),
            "B_im": _w(B_im),
            "C_re": _w(C_re),
            "C_im": _w(C_im),
            "log_dt": _w(log_dt),
            "Dskip": _w(Dskip),
        }
    _B_in = _B_setup()

    return {
        "A_x": _A_in["x"],
        "A_wqkv": _A_in["wqkv"],
        "A_wo": _A_in["wo"],
        "B_u": _B_in["u"],
        "B_A_re": _B_in["A_re"],
        "B_A_im": _B_in["A_im"],
        "B_B_re": _B_in["B_re"],
        "B_B_im": _B_in["B_im"],
        "B_C_re": _B_in["C_re"],
        "B_C_im": _B_in["C_im"],
        "B_log_dt": _B_in["log_dt"],
        "B_Dskip": _B_in["Dskip"],
    }

def reference(A_x, A_wqkv, A_wo, B_u, B_A_re, B_A_im, B_B_re, B_B_im, B_C_re, B_C_im, B_log_dt, B_Dskip):
    def _A_ref(x, wqkv, wo):
        B, S, D = x.shape
        H = 16
        Dh = D // H
        qkv = (lambda x, *d: x.transpose(*d))((x @ wqkv).reshape(B, S, 3, H, Dh), 2, 0, 3, 1, 4)
        q, k, v = qkv[0], qkv[1], qkv[2]
        scores = jnp.einsum("bhqd,bhkd->bhqk", q, k) * (Dh ** -0.5)
        p = _softmax(scores, axis=-1)
        o = jnp.einsum("bhqk,bhkd->bhqd", p, v)
        return (lambda x, *d: x.transpose(*d))(o, 0, 2, 1, 3).reshape(B, S, D) @ wo

    def _B_ref(u, A_re, A_im, B_re, B_im, C_re, C_im, log_dt, Dskip):
        Bsz, L, D = u.shape
        dt = jnp.exp(log_dt)[:, None]
        A = A_re + 1j * A_im
        Bc = B_re + 1j * B_im
        Cc = C_re + 1j * C_im
        logdA = dt * A
        dB = dt * Bc
        l = (lambda x, dt: x.astype(dt))(jnp.arange(L), A_re.dtype)
        P = jnp.exp(logdA[:, :, None] * l[None, None, :])
        K = jnp.einsum("dn,dnl,dn->dl", Cc, P, dB).real
        L2 = 2 * L
        Kp = jnp.pad(K, ((0, 0), (0, L)))
        up = (lambda x, *d: x.transpose(*d))(u, 0, 2, 1)
        up = jnp.pad(up, ((0, 0), (0, 0), (0, L)))
        Kf = (lambda x, axes=(-2,-1): jnp.fft.rfft2(x.astype(jnp.float32), axes=axes))(Kp[:, None, :], axes=(-2, -1))
        Uf = (lambda x, axes=(-2,-1): jnp.fft.rfft2(x.astype(jnp.float32), axes=axes))(up[:, :, None, :], axes=(-2, -1))
        Yf = Uf * Kf[None, :, :, :]
        y = (lambda x, s, axes=(-2,-1): jnp.fft.irfft2(x, s=s, axes=axes).astype(jnp.bfloat16))(Yf, (1, L2), axes=(-2, -1))[:, :, 0, :L]
        y = (lambda x, *d: x.transpose(*d))(y, 0, 2, 1) + u * Dskip[None, None, :]
        return y

    a = _A_ref(A_x, A_wqkv, A_wo)
    b = _B_ref(B_u, B_A_re, B_A_im, B_B_re, B_B_im, B_C_re, B_C_im, B_log_dt, B_Dskip)
    return jnp.concatenate([a, b], axis=-1)
```

```python
import functools

import jax
import jax.numpy as jnp
import numpy as np
import ml_dtypes
import jax.experimental.pallas as pl
import jax.experimental.pallas.tpu as pltpu

F32, BF16 = jnp.float32, jnp.bfloat16
NT = (((1,), (1,)), ((), ()))
TN = (((0,), (0,)), ((), ()))

S, D, H, DH, HP = 2048, 448, 16, 28, 32
L, N, C = 2048, 256, 128
NC = L // C
LOG2E = 1.4426950408889634
TQ = 512
UNR = 8
PG, PD = 3, 3

T2 = list(range(32)) + list(range(32, 64, 2)) + list(range(64, 128, 4)) + list(range(128, 256, 8))
T1 = ([32 * s for s in range(8)] + [256 + 64 * s for s in range(8)]
      + [512 + 128 * s for s in range(8)] + [1024 + 256 * s for s in range(8)])
USED_ROWS = list(range(8)) + list(range(8, 12)) + list(range(16, 20)) + list(range(24, 29))
NCOL = len(T2)


def _tables():
    tl = np.arange(L).astype(np.float32).astype(ml_dtypes.bfloat16).astype(np.int64)
    lut = {}
    for pi, i in enumerate(USED_ROWS):
        s = 1 << (i // 8)
        for jj in range(32):
            lut.setdefault(T1[i] + s * jj, (pi, T2.index(s * jj)))
    X = {}
    for l in range(L):
        pi, j = lut[int(tl[l])]
        c, b = divmod(l, C)
        X.setdefault((pi, c), np.zeros((128, C), np.float32))[j, b] = 1.0
    pairs = sorted(X, key=lambda ic: (ic[1], ic[0]))
    xs = np.stack([X[p] for p in pairs])
    f = np.arange(C + 1)
    b = np.arange(C)
    fc = np.exp(-2j * np.pi * np.outer(b, f) / (2 * C))
    fwd = np.concatenate([fc.real[:, :C], fc.real[:, C:C + 1], fc.imag[:, 1:C]], 1)
    wf = np.where((f == 0) | (f == C), 1.0, 2.0) / (2 * C)
    ic = np.exp(2j * np.pi * np.outer(f, b) / (2 * C)) * wf[:, None]
    invT = np.concatenate([ic.real[:C], ic.real[C:C + 1], -ic.imag[1:C]], 0).T

    def hilo(a):
        h = a.astype(ml_dtypes.bfloat16)
        lo = (a - h.astype(np.float64)).astype(ml_dtypes.bfloat16)
        return np.stack([h, lo])
    return pairs, xs.astype(ml_dtypes.bfloat16), hilo(fwd), hilo(invT)


PAIRS, XS, FHL, FIHL = _tables()

PW_NAMES = ["z1", "z2", "z4", "z8", "z16", "z24", "z32", "z48", "z64", "z96", "z128", "z192",
            "w", "w256", "w512", "w1024"]
PWI = {n: k for k, n in enumerate(PW_NAMES)}


def _split(x):
    h = x.astype(BF16)
    return h, (x - h.astype(F32)).astype(BF16)


def _dot(a, b, dn=None):
    if dn is None:
        return jnp.dot(a, b, preferred_element_type=F32)
    return jax.lax.dot_general(a, b, dn, preferred_element_type=F32)


def _cmul(x, y):
    return x[0] * y[0] - x[1] * y[1], x[0] * y[1] + x[1] * y[0]


def _csq(x):
    return x[0] * x[0] - x[1] * x[1], 2.0 * (x[0] * x[1])


def _attn_body(x_ref, wqT_ref, wk_ref, wvT_ref, wo_ref, o_ref, qT_s, k_s, vT_s, oT_s):
    x = x_ref[0]
    qT = _dot(wqT_ref[...], x, NT)
    qT_s[...] = (qT * (DH ** -0.5 * LOG2E)).astype(BF16)
    vT = _dot(wvT_ref[...], x, NT)
    row = jax.lax.broadcasted_iota(jnp.int32, (H * HP, S), 0)
    vT_s[...] = jnp.where(row % HP == DH, 1.0, vT).astype(BF16)
    k = _dot(x, wk_ref[...]).astype(BF16)
    for h in range(H):
        k_s[h] = k[:, h * HP:(h + 1) * HP]

    def head_body(h, carry):
        kh = k_s[h]
        r0 = pl.multiple_of(h * HP, HP)
        vh = vT_s[pl.ds(r0, HP), :]

        def tile_body(t, c2):
            c0 = pl.multiple_of(t * TQ, TQ)
            qh = qT_s[pl.ds(r0, HP), pl.ds(c0, TQ)]
            sT = _dot(kh, qh)
            m = jnp.max(sT, axis=0, keepdims=True)
            pT = jnp.exp2(sT - m).astype(BF16)
            oT = _dot(vh, pT)
            inv = 1.0 / oT[DH:DH + 1, :]
            rr = jax.lax.broadcasted_iota(jnp.int32, (HP, TQ), 0)
            oT_s[pl.ds(r0, HP), pl.ds(c0, TQ)] = jnp.where(rr < DH, oT * inv, 0.0).astype(BF16)
            return c2
        return jax.lax.fori_loop(0, S // TQ, tile_body, carry)
    jax.lax.fori_loop(0, H, head_body, 0)
    o_ref[0, :, 0:D] = _dot(oT_s[...], wo_ref[...], TN).astype(o_ref.dtype)


def _ssm_body(u_ref, are_ref, aim_ref, bre_ref, bim_ref, cre_ref, cim_ref, ldt_ref, dsk_ref,
              xs_ref, f_ref, fi_ref, o_ref, pw_s, g_s, uf_s, kf_s, yf_s):
    PB = 64

    def pblock(blk, carry):
        rows = pl.ds(pl.multiple_of(blk * PB, PB), PB)
        dt = jnp.exp(ldt_ref[rows, :].astype(F32)).astype(BF16).astype(F32)
        ar = dt * are_ref[rows, :].astype(F32)
        ai = dt * aim_ref[rows, :].astype(F32)
        br = dt * bre_ref[rows, :].astype(F32)
        bi = dt * bim_ref[rows, :].astype(F32)
        w = _cmul((cre_ref[rows, :].astype(F32), cim_ref[rows, :].astype(F32)), (br, bi))

        def cexp(t):
            mag = jnp.exp(ar * t)
            ph = ai * t
            return mag * jnp.cos(ph), mag * jnp.sin(ph)
        z = {1: cexp(1.0), 32: cexp(32.0)}
        for t in (2, 4, 8, 16, 64, 128, 256, 512, 1024):
            z[t] = _csq(z[t // 2])
        z[24] = _cmul(z[16], z[8])
        z[48] = _cmul(z[32], z[16])
        z[96] = _cmul(z[64], z[32])
        z[192] = _cmul(z[128], z[64])
        vals = {"z%d" % t: z[t] for t in (1, 2, 4, 8, 16, 24, 32, 48, 64, 96, 128, 192)}
        vals["w"] = w
        vals["w256"] = _cmul(w, z[256])
        vals["w512"] = _cmul(w, z[512])
        vals["w1024"] = _cmul(w, z[1024])
        for n_, k in PWI.items():
            pw_s[2 * k, rows, :] = vals[n_][0]
            pw_s[2 * k + 1, rows, :] = vals[n_][1]
        return carry
    jax.lax.fori_loop(0, D // PB, pblock, 0)

    sub = jax.lax.broadcasted_iota(jnp.int32, (8, N), 0)
    m1, m2, m4 = (sub & 1) != 0, (sub & 2) != 0, (sub & 4) != 0

    def dstep(it, carry):
        for uu in range(UNR):
            d = it * UNR + uu

            def row(name):
                k = PWI[name]
                return (jnp.broadcast_to(pw_s[2 * k, pl.ds(d, 1), :], (8, N)),
                        jnp.broadcast_to(pw_s[2 * k + 1, pl.ds(d, 1), :], (8, N)))

            def selprod(n1, n2, n4):
                s = lambda m, f: (jnp.where(m, f[0], 1.0), jnp.where(m, f[1], 0.0))
                return _cmul(_cmul(s(m1, row(n1)), s(m2, row(n2))), s(m4, row(n4)))
            zs1 = selprod("z1", "z2", "z4")
            zs2 = _csq(zs1)
            zs4 = _csq(zs2)
            zs8 = _csq(zs4)
            cols = [zs1, _cmul(zs1, row("z8")), _cmul(zs1, row("z16")), _cmul(zs1, row("z24")),
                    _cmul(zs2, row("z32")), _cmul(zs2, row("z48")), _cmul(zs4, row("z64")),
                    _cmul(zs4, row("z96")), _cmul(zs8, row("z128")), _cmul(zs8, row("z192"))]
            zs32 = selprod("z32", "z64", "z128")
            zs64 = _csq(zs32)
            zs128 = _csq(zs64)
            zs256 = _csq(zs128)
            rws = [_cmul(zs32, row("w")), _cmul(zs64, row("w256")), _cmul(zs128, row("w512")),
                   _cmul(zs256, row("w1024"))]
            rhs = jnp.concatenate([jnp.concatenate([c_[0], c_[1]], 1) for c_ in cols], 0)
            lhs = jnp.concatenate([jnp.concatenate([r_[0], -r_[1]], 1) for r_ in rws], 0)
            if PG == 1:
                g = _dot(lhs.astype(BF16), rhs.astype(BF16), NT)
            else:
                lh, ll = _split(lhs)
                rh, rl = _split(rhs)
                g2 = _dot(jnp.concatenate([lh, ll], 0), rh, NT)
                g = g2[:32] + g2[32:] + _dot(lh, rl, NT)
            for pi, i in enumerate(USED_ROWS):
                g_s[pi, pl.ds(d, 1), 0:NCOL] = g[i:i + 1, :]
        return carry
    g_s[:, :, NCOL:128] = jnp.zeros((len(USED_ROWS), D, 128 - NCOL), F32)
    jax.lax.fori_loop(0, D // UNR, dstep, 0)

    fh, fl = f_ref[0], f_ref[1]
    lane = jax.lax.broadcasted_iota(jnp.int32, (D, C), 1)
    sgn = jnp.where(lane % 2 == 0, 1.0, -1.0).astype(F32)
    prev = None
    for c in range(NC):
        kc = None
        for p, (i, cc) in enumerate(PAIRS):
            if cc != c:
                continue
            gh, gl = _split(g_s[i])
            term = _dot(jnp.concatenate([gh, gl], 1), jnp.concatenate([xs_ref[p], xs_ref[p]], 0))
            kc = term if kc is None else kc + term
        if PD == 1:
            kf = _dot(kc.astype(BF16), fh)
        else:
            kh, kl = _split(kc)
            kf = _dot(jnp.concatenate([kh, kh, kl], 1), jnp.concatenate([fh, fl, fh], 0))
        kp = kf if prev is None else kf + jnp.concatenate([sgn, sgn], 1) * prev
        prev = kf
        kr, ki = kp[:, :C], kp[:, C:]
        kf_s[c, 0] = kr
        kf_s[c, 1] = jnp.where(lane == 0, 0.0, ki)
        kf_s[c, 2] = jnp.where(lane == 0, ki, kr)
        uc = u_ref[0, c * C:(c + 1) * C, :]
        if PD == 1:
            uf = _dot(uc, fh, TN)
        else:
            uf = _dot(jnp.concatenate([uc, uc], 0), jnp.concatenate([fh, fl], 0), TN)
        uf_s[c, 0] = uf[:, :C]
        uf_s[c, 1] = uf[:, C:]

    RB = 64
    fih, fil = fi_ref[0], fi_ref[1]
    dsk = dsk_ref[...].astype(F32)

    def chunk_out(a, carry):
        def rblock(rb, c2):
            rows = pl.ds(pl.multiple_of(rb * RB, RB), RB)

            def mac(dl, acc):
                yr, yi = acc
                ur = uf_s[a - dl, 0, rows, :]
                ui = uf_s[a - dl, 1, rows, :]
                kr = kf_s[dl, 0, rows, :]
                kz = kf_s[dl, 1, rows, :]
                kb = kf_s[dl, 2, rows, :]
                return yr + (ur * kr - ui * kz), yi + (ur * kz + ui * kb)
            z = jnp.zeros((RB, C), F32)
            yr, yi = jax.lax.fori_loop(0, a + 1, mac, (z, z))
            yf_s[rows, 0:C] = yr
            yf_s[rows, C:2 * C] = yi
            return c2
        jax.lax.fori_loop(0, D // RB, rblock, 0)
        yf = yf_s[...]
        if PD == 1:
            y = _dot(fih, yf.astype(BF16), NT)
        else:
            yh, yl = _split(yf)
            y = _dot(jnp.concatenate([fih, fil, fih], 1), jnp.concatenate([yh, yh, yl], 1), NT)
        r0 = pl.multiple_of(a * C, C)
        uc = u_ref[0, pl.ds(r0, C), :].astype(F32)
        res = y.astype(BF16).astype(F32) + (uc * dsk).astype(BF16).astype(F32)
        o_ref[0, pl.ds(r0, C), D:2 * D] = res.astype(o_ref.dtype)
        return carry
    jax.lax.fori_loop(0, NC, chunk_out, 0)


def _kernel(x_ref, wqT_ref, wk_ref, wvT_ref, wo_ref,
            u_ref, are_ref, aim_ref, bre_ref, bim_ref, cre_ref, cim_ref, ldt_ref, dsk_ref,
            xs_ref, f_ref, fi_ref, o_ref,
            qT_s, k_s, vT_s, oT_s, pw_s, g_s, uf_s, kf_s, yf_s):
    _attn_body(x_ref, wqT_ref, wk_ref, wvT_ref, wo_ref, o_ref, qT_s, k_s, vT_s, oT_s)
    _ssm_body(u_ref, are_ref, aim_ref, bre_ref, bim_ref, cre_ref, cim_ref, ldt_ref, dsk_ref,
              xs_ref, f_ref, fi_ref, o_ref, pw_s, g_s, uf_s, kf_s, yf_s)


@jax.jit
def pallas_concat_heads__mha_block__ssm_conv_s4__prompt_kernel(
    A_x: jax.Array,
    A_wqkv: jax.Array,
    A_wo: jax.Array,
    B_u: jax.Array,
    B_A_re: jax.Array,
    B_A_im: jax.Array,
    B_B_re: jax.Array,
    B_B_im: jax.Array,
    B_C_re: jax.Array,
    B_C_im: jax.Array,
    B_log_dt: jax.Array,
    B_Dskip: jax.Array,
):
    w = jnp.pad(A_wqkv.reshape(D, 3, H, DH), ((0, 0), (0, 0), (0, 0), (0, HP - DH)))
    wqT = w[:, 0].reshape(D, H * HP).T
    wk = w[:, 1].reshape(D, H * HP)
    wvT = w[:, 2].reshape(D, H * HP).T
    wop = jnp.pad(A_wo.reshape(H, DH, D), ((0, 0), (0, HP - DH), (0, 0))).reshape(H * HP, D)
    scratch = [
        pltpu.VMEM((H * HP, S), BF16), pltpu.VMEM((H, S, HP), BF16),
        pltpu.VMEM((H * HP, S), BF16), pltpu.VMEM((H * HP, S), BF16),
        pltpu.VMEM((2 * len(PW_NAMES), D, N), F32), pltpu.VMEM((len(USED_ROWS), D, 128), F32),
        pltpu.VMEM((NC, 2, D, C), F32), pltpu.VMEM((NC, 3, D, C), F32), pltpu.VMEM((D, 2 * C), F32),
    ]
    return pl.pallas_call(
        _kernel,
        out_shape=jax.ShapeDtypeStruct((1, S, 2 * D), BF16),
        scratch_shapes=scratch,
        compiler_params=pltpu.CompilerParams(vmem_limit_bytes=110 * 1024 * 1024),
    )(A_x, wqT, wk, wvT, wop,
      B_u, B_A_re, B_A_im, B_B_re, B_B_im, B_C_re, B_C_im,
      B_log_dt.reshape(D, 1), B_Dskip.reshape(1, D),
      jnp.asarray(XS), jnp.asarray(FHL), jnp.asarray(FIHL))
```

```python
import jax
import jax.numpy as jnp
import numpy as np
import ml_dtypes
import jax.experimental.pallas as pl
import jax.experimental.pallas.tpu as pltpu

F32, BF16 = jnp.float32, jnp.bfloat16
NT = (((1,), (1,)), ((), ()))
TN = (((0,), (0,)), ((), ()))

S, D, H, DH, HP = 2048, 448, 16, 28, 32
L, N, C = 2048, 256, 128
NC = L // C
LOG2E = 1.4426950408889634
TQ = 1024
UNR = 28
N1 = 448 // UNR
N2 = 14
PG, PD = 1, 1

T2 = list(range(32)) + list(range(32, 64, 2)) + list(range(64, 128, 4)) + list(range(128, 256, 8))
T1 = ([32 * s for s in range(8)] + [256 + 64 * s for s in range(8)]
      + [512 + 128 * s for s in range(8)] + [1024 + 256 * s for s in range(8)])
USED_ROWS = list(range(8)) + list(range(8, 12)) + list(range(16, 20)) + list(range(24, 29))
NCOL = len(T2)


def _tables():
    tl = np.arange(L).astype(np.float32).astype(ml_dtypes.bfloat16).astype(np.int64)
    lut = {}
    for pi, i in enumerate(USED_ROWS):
        s = 1 << (i // 8)
        for jj in range(32):
            lut.setdefault(T1[i] + s * jj, (pi, T2.index(s * jj)))
    X = {}
    for l in range(L):
        pi, j = lut[int(tl[l])]
        c, b = divmod(l, C)
        X.setdefault((pi, c), np.zeros((128, C), np.float32))[j, b] = 1.0
    pairs = sorted(X, key=lambda ic: (ic[1], ic[0]))
    xs = np.stack([X[p] for p in pairs])
    f = np.arange(C + 1)
    b = np.arange(C)
    fc = np.exp(-2j * np.pi * np.outer(b, f) / (2 * C))
    fwd = np.concatenate([fc.real[:, :C], fc.real[:, C:C + 1], fc.imag[:, 1:C]], 1)
    wf = np.where((f == 0) | (f == C), 1.0, 2.0) / (2 * C)
    ic = np.exp(2j * np.pi * np.outer(f, b) / (2 * C)) * wf[:, None]
    invT = np.concatenate([ic.real[:C], ic.real[C:C + 1], -ic.imag[1:C]], 0).T

    def hilo(a):
        h = a.astype(ml_dtypes.bfloat16)
        lo = (a - h.astype(np.float64)).astype(ml_dtypes.bfloat16)
        return np.stack([h, lo])
    return pairs, xs.astype(ml_dtypes.bfloat16), hilo(fwd), hilo(invT)


PAIRS, XS, FHL, FIHL = _tables()

PW_NAMES = ["z1", "z2", "z4", "z8", "z16", "z24", "z32", "z48", "z64", "z96", "z128", "z192",
            "w", "w256", "w512", "w1024"]
PWI = {n: k for k, n in enumerate(PW_NAMES)}


def _split(x):
    h = x.astype(BF16)
    return h, (x - h.astype(F32)).astype(BF16)


def _dot(a, b, dn=None):
    if dn is None:
        return jnp.dot(a, b, preferred_element_type=F32)
    return jax.lax.dot_general(a, b, dn, preferred_element_type=F32)


def _cmul(x, y):
    return x[0] * y[0] - x[1] * y[1], x[0] * y[1] + x[1] * y[0]


def _csq(x):
    return x[0] * x[0] - x[1] * x[1], 2.0 * (x[0] * x[1])


def _pad_heads(w, axis):
    pieces = []
    zshape = list(w.shape)
    zshape[axis] = HP - DH
    z = jnp.zeros(zshape, w.dtype)
    for h in range(H):
        pieces.append(jax.lax.slice_in_dim(w, h * DH, (h + 1) * DH, axis=axis))
        pieces.append(z)
    return jnp.concatenate(pieces, axis=axis)


def _attn_proj(xT_ref, wqkv_ref, qT_s, k_s, vT_s):
    xT = xT_ref[...]
    wq = _pad_heads(wqkv_ref[:, 0:D], 1)
    qT_s[...] = (_dot(wq, xT, TN) * (DH ** -0.5 * LOG2E)).astype(BF16)
    wv = _pad_heads(wqkv_ref[:, 2 * D:3 * D], 1)
    vT = _dot(wv, xT, TN)
    row = jax.lax.broadcasted_iota(jnp.int32, (H * HP, S), 0)
    vT_s[...] = jnp.where(row % HP == DH, 1.0, vT).astype(BF16)
    wk = _pad_heads(wqkv_ref[:, D:2 * D], 1)
    kT = _dot(wk, xT, TN)
    for h in range(H):
        k_s[h] = kT[h * HP:(h + 1) * HP, :].T.astype(BF16)


NTILE = S // TQ
TOTAL = H * NTILE


NSUB = 4
KS = S // NSUB


def _attn_scores(i, slot, qT_s, k_s, s_buf, m_buf, j):
    h = i // NTILE
    t = i % NTILE
    r0 = pl.multiple_of(h * HP, HP)
    c0 = pl.multiple_of(t * TQ, TQ)
    sT = _dot(k_s[h, j * KS:(j + 1) * KS, :], qT_s[pl.ds(r0, HP), pl.ds(c0, TQ)])
    s_buf[slot, j * KS:(j + 1) * KS, :] = sT
    m = jnp.max(sT, axis=0, keepdims=True)
    m_buf[slot] = m if j == 0 else jnp.maximum(m_buf[slot], m)


def _attn_finish(i, slot, vT_s, oT_s, s_buf, m_buf, acc_s, j):
    h = i // NTILE
    t = i % NTILE
    r0 = pl.multiple_of(h * HP, HP)
    c0 = pl.multiple_of(t * TQ, TQ)
    pT = jnp.exp2(s_buf[slot, j * KS:(j + 1) * KS, :] - m_buf[slot]).astype(BF16)
    oT = _dot(vT_s[pl.ds(r0, HP), j * KS:(j + 1) * KS], pT)
    if j > 0:
        oT = oT + acc_s[...]
    if j < NSUB - 1:
        acc_s[...] = oT
    else:
        inv = 1.0 / oT[DH:DH + 1, :]
        rr = jax.lax.broadcasted_iota(jnp.int32, (HP, TQ), 0)
        oT_s[pl.ds(r0, HP), pl.ds(c0, TQ)] = jnp.where(rr < DH, oT * inv, 0.0).astype(BF16)


def _attn_out(wo_ref, o_ref, oT_s):
    wo = _pad_heads(wo_ref[...], 0)
    o_ref[:, 0:D] = _dot(oT_s[...], wo, TN).astype(o_ref.dtype)


def _ssm_pow(are_ref, aim_ref, bre_ref, bim_ref, cre_ref, cim_ref, ldt_ref, pw_s):
    PB = 64

    def pblock(blk, carry):
        rows = pl.ds(pl.multiple_of(blk * PB, PB), PB)
        dt = jnp.exp(ldt_ref[rows, :].astype(F32)).astype(BF16).astype(F32)
        ar = dt * are_ref[rows, :].astype(F32)
        ai = dt * aim_ref[rows, :].astype(F32)
        br = dt * bre_ref[rows, :].astype(F32)
        bi = dt * bim_ref[rows, :].astype(F32)
        w = _cmul((cre_ref[rows, :].astype(F32), cim_ref[rows, :].astype(F32)), (br, bi))

        def cexp(t):
            mag = jnp.exp(ar * t)
            ph = ai * t
            return mag * jnp.cos(ph), mag * jnp.sin(ph)
        z = {1: cexp(1.0)}
        for t in (2, 4, 8, 16, 32, 64, 128, 256, 512, 1024):
            z[t] = _csq(z[t // 2])
        z[24] = _cmul(z[16], z[8])
        z[48] = _cmul(z[32], z[16])
        z[96] = _cmul(z[64], z[32])
        z[192] = _cmul(z[128], z[64])
        vals = {"z%d" % t: z[t] for t in (1, 2, 4, 8, 16, 24, 32, 48, 64, 96, 128, 192)}
        vals["w"] = w
        vals["w256"] = _cmul(w, z[256])
        vals["w512"] = _cmul(w, z[512])
        vals["w1024"] = _cmul(w, z[1024])
        for n_, k in PWI.items():
            pw_s[2 * k, rows, :] = vals[n_][0]
            pw_s[2 * k + 1, rows, :] = vals[n_][1]
        return carry
    with jax.named_scope("b_pow"):
        jax.lax.fori_loop(0, D // PB, pblock, 0)


def _ssm_perd(it, pw_s, g_s, u0=0, u1=UNR):
    sub = jax.lax.broadcasted_iota(jnp.int32, (8, N), 0)
    m1, m2, m4 = (sub & 1) != 0, (sub & 2) != 0, (sub & 4) != 0

    def dstep(it, carry):
        for uu in range(u0, u1):
            d = it * UNR + uu

            def row(name):
                k = PWI[name]
                return (jnp.broadcast_to(pw_s[2 * k, pl.ds(d, 1), :], (8, N)),
                        jnp.broadcast_to(pw_s[2 * k + 1, pl.ds(d, 1), :], (8, N)))

            def selprod(n1, n2, n4):
                s = lambda m, f: (jnp.where(m, f[0], 1.0), jnp.where(m, f[1], 0.0))
                return _cmul(_cmul(s(m1, row(n1)), s(m2, row(n2))), s(m4, row(n4)))
            zs1 = selprod("z1", "z2", "z4")
            zs2 = _csq(zs1)
            zs4 = _csq(zs2)
            zs8 = _csq(zs4)
            cols = [zs1, _cmul(zs1, row("z8")), _cmul(zs1, row("z16")), _cmul(zs1, row("z24")),
                    _cmul(zs2, row("z32")), _cmul(zs2, row("z48")), _cmul(zs4, row("z64")),
                    _cmul(zs4, row("z96")), _cmul(zs8, row("z128")), _cmul(zs8, row("z192"))]
            zs32 = selprod("z32", "z64", "z128")
            zs64 = _csq(zs32)
            zs128 = _csq(zs64)
            zs256 = _csq(zs128)
            rws = [_cmul(zs32, row("w")), _cmul(zs64, row("w256")), _cmul(zs128, row("w512")),
                   _cmul(zs256, row("w1024"))]
            rhs = jnp.concatenate([jnp.concatenate([c_[0], c_[1]], 1) for c_ in cols], 0)
            lhs = jnp.concatenate([jnp.concatenate([r_[0], -r_[1]], 1) for r_ in rws], 0)
            if PG == 1:
                g = _dot(lhs.astype(BF16), rhs.astype(BF16), NT)
            else:
                lh, ll = _split(lhs)
                rh, rl = _split(rhs)
                g2 = _dot(jnp.concatenate([lh, ll], 0), rh, NT)
                g = g2[:32] + g2[32:] + _dot(lh, rl, NT)
            for pi, i in enumerate(USED_ROWS):
                g_s[pi, pl.ds(d, 1), 0:NCOL] = g[i:i + 1, :]
        return carry
    dstep(it, 0)


def _ssm_dft(uT_ref, xs_ref, f_ref, g_s, uf_s, kf_s):
    fh, fl = f_ref[0], f_ref[1]
    lane = jax.lax.broadcasted_iota(jnp.int32, (D, C), 1)
    sgn = jnp.where(lane % 2 == 0, 1.0, -1.0).astype(F32)
    prev = None
    for c in range(NC):
        kc = None
        for p, (i, cc) in enumerate(PAIRS):
            if cc != c:
                continue
            if PD == 1:
                term = _dot(g_s[i].astype(BF16), xs_ref[p])
            else:
                gh, gl = _split(g_s[i])
                term = _dot(jnp.concatenate([gh, gl], 1), jnp.concatenate([xs_ref[p], xs_ref[p]], 0))
            kc = term if kc is None else kc + term
        if PD == 1:
            kf = _dot(kc.astype(BF16), fh)
        else:
            kh, kl = _split(kc)
            kf = _dot(jnp.concatenate([kh, kh, kl], 1), jnp.concatenate([fh, fl, fh], 0))
        kp = kf if prev is None else kf + jnp.concatenate([sgn, sgn], 1) * prev
        prev = kf
        kr, ki = kp[:, :C], kp[:, C:]
        kf_s[c, 0] = kr
        kf_s[c, 1] = jnp.where(lane == 0, 0.0, ki)
        kf_s[c, 2] = jnp.where(lane == 0, ki, kr)
        uc = uT_ref[:, c * C:(c + 1) * C]
        if PD == 1:
            uf = _dot(uc, fh)
        else:
            uf = _dot(jnp.concatenate([uc, uc], 1), jnp.concatenate([fh, fl], 0))
        uf_s[c, 0] = uf[:, :C]
        uf_s[c, 1] = uf[:, C:]


MAC_SPLIT = [range(0, 8), range(8, 11), range(11, 14), range(14, 16)]


def _ssm_mac(rb, uf_s, kf_s, yf_s, part):
    RB = 32

    def rblock(rb, c2):
        rows = pl.ds(pl.multiple_of(rb * RB, RB), RB)
        for a in MAC_SPLIT[part]:
            yr = yi = None
            for dl in range(a + 1):
                ur = uf_s[a - dl, 0, rows, :]
                ui = uf_s[a - dl, 1, rows, :]
                kr = kf_s[dl, 0, rows, :]
                kz = kf_s[dl, 1, rows, :]
                kb = kf_s[dl, 2, rows, :]
                tr = ur * kr - ui * kz
                ti = ur * kz + ui * kb
                yr = tr if yr is None else yr + tr
                yi = ti if yi is None else yi + ti
            yf_s[a, rows, 0:C] = yr
            yf_s[a, rows, C:2 * C] = yi
        return c2
    rblock(rb, 0)


def _ssm_inv(uT_ref, dsk_ref, fi_ref, o_ref, emit_rows, yf_s):
    fih, fil = fi_ref[0], fi_ref[1]
    dsk = dsk_ref[...].astype(F32)

    def chunk_out(a, carry):
        yf = yf_s[a]
        if PD == 1:
            y = _dot(fih, yf.astype(BF16), NT)
        else:
            yh, yl = _split(yf)
            y = _dot(jnp.concatenate([fih, fil, fih], 1), jnp.concatenate([yh, yh, yl], 1), NT)
        r0 = pl.multiple_of(a * C, C)
        uc = uT_ref[:, pl.ds(r0, C)].astype(F32).T
        res = y.astype(BF16).astype(F32) + (uc * dsk).astype(BF16).astype(F32)
        o_ref[pl.ds(r0, C), D:2 * D] = res.astype(o_ref.dtype)
        emit_rows(a)
        return carry
    with jax.named_scope("b_inv"):
        jax.lax.fori_loop(0, NC, chunk_out, 0)


_IN_SHAPES = [
    ((D, S), BF16), ((D, 3 * D), BF16), ((D, D), BF16),
    ((D, L), BF16),
    ((D, N), BF16), ((D, N), BF16), ((D, N), BF16), ((D, N), BF16), ((D, N), BF16), ((D, N), BF16),
    ((D, 1), BF16), ((1, D), BF16),
    (XS.shape, BF16), (FHL.shape, BF16), (FIHL.shape, BF16),
]
_NIN = len(_IN_SHAPES)


def _kernel(*refs):
    hbm_in = refs[:_NIN]
    out_hbm = refs[_NIN]
    vm_in = refs[_NIN + 1:2 * _NIN + 1]
    (o_s, qT_s, k_s, vT_s, oT_s, s_buf, m_buf, acc_s, pw_s, g_s, uf_s, kf_s, yf_s,
     in_sems, out_sems) = refs[2 * _NIN + 1:]

    copies = []
    for i in range(_NIN):
        src = hbm_in[i].at[0] if i in (0, 3) else hbm_in[i]
        copies.append(pltpu.make_async_copy(src, vm_in[i], in_sems.at[i]))
    for cp in copies[4:11] + copies[:4] + copies[11:]:
        cp.start()
    (xT_r, wqkv_r, wo_r, uT_r, are_r, aim_r, bre_r, bim_r, cre_r, cim_r, ldt_r, dsk_r,
     xs_r, f_r, fi_r) = vm_in
    for cp in copies[4:11]:
        cp.wait()
    _ssm_pow(are_r, aim_r, bre_r, bim_r, cre_r, cim_r, ldt_r, pw_s)
    g_s[:, :, NCOL:128] = jnp.zeros((len(USED_ROWS), D, 128 - NCOL), F32)
    for cp in copies[:3]:
        cp.wait()
    with jax.named_scope("a_proj"):
        _attn_proj(xT_r, wqkv_r, qT_s, k_s, vT_s)
    for cp in copies[3:4] + copies[11:]:
        cp.wait()

    def sc(i, j):
        _attn_scores(i, i % 2, qT_s, k_s, s_buf, m_buf, j)

    def fin(i, j):
        _attn_finish(i, i % 2, vT_s, oT_s, s_buf, m_buf, acc_s, j)

    def body1(i, c):
        for j in range(NSUB):
            sc(i + 1, j)
            _ssm_perd(i, pw_s, g_s, j * UNR // NSUB, (2 * j + 1) * UNR // (2 * NSUB))
            fin(i, j)
            _ssm_perd(i, pw_s, g_s, (2 * j + 1) * UNR // (2 * NSUB), (j + 1) * UNR // NSUB)
        return c

    def body2(i, c):
        for j in range(NSUB):
            sc(i + 1, j)
            fin(i, j)
            _ssm_mac(i - N1, uf_s, kf_s, yf_s, j)
        return c

    def body3(i, c):
        for j in range(NSUB):
            sc(i + 1, j)
            fin(i, j)
        return c

    for j in range(NSUB):
        sc(0, j)
    with jax.named_scope("loop1_perd"):
        jax.lax.fori_loop(0, N1, body1, 0)
    with jax.named_scope("b_dft"):
        _ssm_dft(uT_r, xs_r, f_r, g_s, uf_s, kf_s)
    with jax.named_scope("loop2_mac"):
        jax.lax.fori_loop(N1, N1 + N2, body2, 0)
    with jax.named_scope("loop3"):
        jax.lax.fori_loop(N1 + N2, TOTAL - 1, body3, 0)
        for j in range(NSUB):
            fin(TOTAL - 1, j)
    with jax.named_scope("a_out"):
        _attn_out(wo_r, o_s, oT_s)

    def out_copy(a):
        r0 = pl.multiple_of(a * C, C)
        return pltpu.make_async_copy(o_s.at[pl.ds(r0, C), :], out_hbm.at[0, pl.ds(r0, C), :], out_sems.at[a])

    def emit_rows(a):
        out_copy(a).start()

    _ssm_inv(uT_r, dsk_r, fi_r, o_s, emit_rows, yf_s)
    for a in range(NC):
        out_copy(a).wait()


@jax.jit
def pallas_concat_heads__mha_block__ssm_conv_s4__prompt_kernel(
    A_x: jax.Array,
    A_wqkv: jax.Array,
    A_wo: jax.Array,
    B_u: jax.Array,
    B_A_re: jax.Array,
    B_A_im: jax.Array,
    B_B_re: jax.Array,
    B_B_im: jax.Array,
    B_C_re: jax.Array,
    B_C_im: jax.Array,
    B_log_dt: jax.Array,
    B_Dskip: jax.Array,
):
    scratch = [pltpu.VMEM(shp, dt) for shp, dt in _IN_SHAPES] + [
        pltpu.VMEM((S, 2 * D), BF16),
        pltpu.VMEM((H * HP, S), BF16), pltpu.VMEM((H, S, HP), BF16),
        pltpu.VMEM((H * HP, S), BF16), pltpu.VMEM((H * HP, S), BF16),
        pltpu.VMEM((2, S, TQ), F32), pltpu.VMEM((2, 1, TQ), F32), pltpu.VMEM((HP, TQ), F32),
        pltpu.VMEM((2 * len(PW_NAMES), D, N), F32), pltpu.VMEM((len(USED_ROWS), D, 128), F32),
        pltpu.VMEM((NC, 2, D, C), F32), pltpu.VMEM((NC, 3, D, C), F32), pltpu.VMEM((NC, D, 2 * C), F32),
        pltpu.SemaphoreType.DMA((_NIN,)), pltpu.SemaphoreType.DMA((NC,)),
    ]
    return pl.pallas_call(
        _kernel,
        out_shape=jax.ShapeDtypeStruct((1, S, 2 * D), BF16),
        in_specs=[pl.BlockSpec(memory_space=pl.ANY)] * _NIN,
        out_specs=pl.BlockSpec(memory_space=pl.ANY),
        scratch_shapes=scratch,
        compiler_params=pltpu.CompilerParams(vmem_limit_bytes=120 * 1024 * 1024),
    )(jnp.transpose(A_x, (0, 2, 1)), A_wqkv, A_wo,
      jnp.transpose(B_u, (0, 2, 1)), B_A_re, B_A_im, B_B_re, B_B_im, B_C_re, B_C_im,
      B_log_dt.reshape(D, 1), B_Dskip.reshape(1, D),
      jnp.asarray(XS), jnp.asarray(FHL), jnp.asarray(FIHL))
```
